```python
import os as _os
_os.environ.setdefault("JAX_PLATFORMS", "cpu")
import jax
import jax.numpy as jnp

def _softmax(x, axis=-1):
    return jax.nn.softmax(x, axis=axis)
def _gelu(x):
    return jax.nn.gelu(x, approximate=True)
def _silu(x):
    return jax.nn.silu(x)
def _sigmoid(x):
    return jax.nn.sigmoid(x)
def _layernorm(x, axis=-1, eps=1e-5):
    m = jnp.mean(x, axis=axis, keepdims=True)
    v = jnp.var(x, axis=axis, keepdims=True)
    return (x - m) / jnp.sqrt(v + eps)
def _scatter_add(tgt, idx, src, axis=0):
    return tgt.at[idx].add(src)
def _segment_sum(src, seg, n):
    return jax.ops.segment_sum(src, seg, n)
class _Rng:
    def __init__(self, key):
        self._k = key
    def _next(self):
        self._k, sub = jax.random.split(self._k)
        return sub
    def normal(self, shape):
        return jax.random.normal(self._next(), shape, dtype=jnp.bfloat16)
    def randint(self, lo, hi, shape):
        return jax.random.randint(self._next(), shape, lo, hi, dtype=jnp.int32)
    def uniform(self, shape, lo=0.0, hi=1.0):
        return jax.random.uniform(self._next(), shape, jnp.bfloat16, lo, hi)
    def permutation(self, n):
        return jax.random.permutation(self._next(), n)


kernel_name = 'standalone__fft_conv__vision'

def setup_inputs():
    _rng = _Rng(jax.random.key(int.from_bytes(__import__("os").urandom(4), "little")))
    _w = (lambda a: (lambda t: t.astype(jnp.bfloat16) if jnp.issubdtype(t.dtype, jnp.floating) else t)(jnp.asarray(a)))
    H = W = 224
    C = 96
    K = 3
    return {
        "x": _w((lambda *s: _rng.normal(s) * 0.05)(1, H, W, C)),
        "w": _w((lambda *s: _rng.normal(s) * 0.05)(K, K, C, C)),
    }

def reference(x, w):
    B, H, W, C = x.shape
    K = w.shape[0]
    wp = jnp.pad(w, ((0, H - K), (0, W - K), (0, 0), (0, 0)))
    Xf = (lambda x, axes=(-2,-1): jnp.fft.rfft2(x.astype(jnp.float32), axes=axes))(x, axes=(1, 2))
    Wf = (lambda x, axes=(-2,-1): jnp.fft.rfft2(x.astype(jnp.float32), axes=axes))(wp, axes=(0, 1))
    Yf = jnp.einsum('bhwi,hwio->bhwo', Xf, Wf)
    y = (lambda x, s, axes=(-2,-1): jnp.fft.irfft2(x, s=s, axes=axes).astype(jnp.bfloat16))(Yf, (H, W), axes=(1, 2))
    return y
```

```python
import functools
import jax, jax.numpy as jnp, numpy as np
from jax import lax
from jax.experimental import pallas as pl
from jax.experimental.pallas import tpu as pltpu

H = W = 224
C = 96
F32 = jnp.float32
BF16 = jnp.bfloat16
U32 = jnp.uint32
A = float(2.0 ** -0.5)
B = float(2.0 ** 0.5)

def _weight_coefs():
    pts = [0.0, A, -A, B, -B]
    G = np.zeros((6, 3))
    for j, p in enumerate(pts):
        n = np.prod([p - q for l, q in enumerate(pts) if l != j])
        G[j] = [p ** i / n for i in range(3)]
    G[5, 2] = 1.0
    G[1:5] *= 0.5
    return np.round(G, 12)
G = _weight_coefs()

NGRP, NT = 5, 9
def _tiles():
    tiles, cur, room, s = [], [], 128, 2
    for g in range(NGRP):
        end = s + W
        while s < end:
            e = min(end, s + room - 2)
            cur.append((g, s, e))
            room -= e - s + 2
            s = e
            if room == 0:
                tiles.append(cur)
                cur, room = [], 128
        s = (s + 2) % 128
    tiles.append(cur)
    assert len(tiles) == NT
    return tiles
TILES = _tiles()

def _runs(owner):
    keys = []
    for k in owner:
        if k is not None and k not in keys:
            keys.append(k)
    return keys

def as_bf16(v): return pltpu.bitcast(v, BF16)
def as_u32(v): return pltpu.bitcast(v, U32)
def as_f32(v): return pltpu.bitcast(v, F32)
def mm(a, b): return jnp.dot(a, b, preferred_element_type=F32)

XR = H + 10
XS, RS = 0, XR
TR = 2 * XR
YS = TR + 24
PS = YS + 4 * NT
US = PS + 4
PR = US + 14
PC = PR + 12
NROWS = PC + 1
LO = slice(0, 128)
HI = slice(128, 224)

def make(n1=5, wdyn=None, flags=None, skip="",
         d_lhs=12, d_rot=27, d_raw=16, d_tf=2, d_p=2, d_fix=11, pre=(1, 2, 3, 4), tf0=0, tfs=4,
         rpos=(24 * 1 + 2, 24 * 3 + 2, 24 * 5 + 2, 24 * 7 + 0, 24 * 8 + 2), apos=(0, 24 * 1 + 16, 24 * 3 + 16, 24 * 5 + 16, 24 * 7 + 14),
         quant=2, pace=2, wfirst=False, wprio=False, wset=(0, 1, 2, 3, 4)):
    nit = (H // 4 - 1) // NGRP
    rows_it = 4 * NGRP
    nr = nit if wdyn else n1

    def kernel(x_hbm, w_hbm, o_hbm, ws, ob, w_ref, z_ref, sem):
        ws_b = ws.bitcast(BF16)
        ob_b = ob.bitcast(BF16)
        def st16(row, rows, v):
            ws_b[pl.ds(row, 1), rows, LO] = v[None].astype(BF16)
        def rd(s, d, n, sm):
            if 'r' in skip: return ()
            return (pltpu.make_async_copy(x_hbm.at[pl.ds(s, n)], ws_b.at[pl.ds(XS + d, n)], sm),)
        def wr(s, n):
            if 'w' in skip: return ()
            return (pltpu.make_async_copy(ob_b.at[pl.ds(s, n)], o_hbm.at[pl.ds(s, n)], sem.at[0]),)
        def start(cs, prio=0):
            for c in cs: c.start(priority=prio)
        def wait(cs):
            for c in cs: c.wait()

        def cs(i): return pl.ds(8 * i, 8)
        def cb(i): return pl.ds(16 * i, 16)

        def merge(owner, load):
            last = next(k for k in owner if k is not None)
            runs = []
            for l, k in enumerate(owner):
                last = last if k is None else k
                if not runs or runs[-1][0] != last:
                    runs.append([last, l, l])
                runs[-1][2] = l + 1
            vals = {}
            for k, _, _ in runs:
                if k not in vals:
                    vals[k] = load(k)
            if len(runs) == 3 and runs[0][0] == runs[2][0]:
                lane = lax.broadcasted_iota(jnp.int32, (8, 128), 1)
                return jnp.where((lane >= runs[1][1]) & (lane < runs[1][2]), vals[runs[1][0]], vals[runs[0][0]])
            return jnp.concatenate([vals[k][:, a:b] for k, a, b in runs], axis=1)

        def transform(d):
            d = [as_bf16(v).astype(F32) for v in d]
            r = d[4] - d[2]
            e1 = r - d[2]
            e2 = r + d[4]
            q = d[3] - d[1]
            o1 = A * (q - d[1])
            o2 = B * (q + d[3])
            return [(d[0] + d[4]) - 2.5 * d[2], e1 + o1, e1 - o1, e2 + o2, e2 - o2, (d[1] + d[5]) - 2.5 * d[3]]

        def weights():
            eye = (lax.broadcasted_iota(jnp.int32, (C, C), 0) == lax.broadcasted_iota(jnp.int32, (C, C), 1)).astype(BF16)
            def tr(m):
                return lax.dot_general(eye, m, (((1,), (1,)), ((), ())), preferred_element_type=F32)
            for e in range(2):
                f = [tr(jnp.concatenate([w_ref[2 - i, 0, 32 * e:32 * e + 32, :], w_ref[2 - i, 1 + e]], axis=0)) for i in range(3)]
                for j in range(6):
                    acc = None
                    for i in (0, 2, 1):
                        if G[j, i] != 0.0:
                            t = f[i] if abs(G[j, i]) == 1.0 else f[i] * abs(float(G[j, i]))
                            acc = (t if G[j, i] > 0 else -t) if acc is None else (acc + t if G[j, i] > 0 else acc - t)
                    st16(US + 2 * j + e, slice(None), acc)
            z = jnp.zeros((32, C), BF16)
            rem = [w_ref[2 - i, 0, 64:96, :] for i in range(3)]
            st16(US + 12, slice(None), tr(jnp.concatenate(rem + [z], axis=0)))
            st16(US + 13, slice(None), tr(jnp.concatenate([z] + rem, axis=0)))

        def tile_inputs(n, i, hl, gmin):
            owner = [None] * 128
            for g, s, e in TILES[n % NT]:
                g += NGRP * (n // NT)
                if g >= gmin:
                    for w in range(s - 2, e):
                        owner[w % 128] = (g, 0 if w < 128 else 1 if w < W else 2)
            def load(q, key):
                g, kind = key
                return ws[hl + ((RS if kind == 2 else XS) + 4 * g + q), cs(i), HI if kind == 1 else LO]
            return [merge(owner, functools.partial(load, q)) for q in range(6)], owner

        def store_tile(n, i, d, ts, zs):
            base = TR + 8 * (n % 3)
            for j in range(6):
                st16(zs + (base + j), cb(i), ts[j])
            if i >= 4:
                for q in range(6):
                    ws[zs + (base + 6 + q // 3), cs(2 * (q % 3) + i - 4), LO] = d[q]

        def assemble_load(g, k, i, zl):
            direct, wrapped, hi = [None] * 128, [None] * 128, None
            for n, segs in enumerate(TILES):
                for gg, s, e in segs:
                    if gg == g:
                        for w in range(s, e):
                            if w < 128: direct[w] = n
                            elif w < W:
                                assert hi in (None, n)
                                hi = n
                            else:
                                wrapped[w % 128] = n
                                direct[w - W] = "wrap"
            vals = {}
            def load(n):
                if n not in vals:
                    vals[n] = ws[zl + (YS + 4 * n + k), cs(i), LO]
                return vals[n]
            rolled = pltpu.roll(merge(wrapped, load), 32, 1)
            nwrap = direct.count("wrap")
            return merge([None] * nwrap + direct[nwrap:], load), load(hi)[:, 0:96], rolled[:, 0:nwrap], list(vals)

        def run(first, gmin, h0, zl, zs, write):
            hl = h0 + zl
            hs = h0 + zs
            acts = []
            log = []
            def at(pos, prio, fn):
                assert pos < 24 * NT + 1, pos
                pos -= 24 * first
                acts.append((pos // quant if pos >= 0 else -1, prio if pos >= 0 else 0, pos, len(acts), fn))
            for n in range(first, NT):
                t0 = 24 * n
                st = {}
                tb = TR + 8 * (n % 3)
                def sched_main(j, k, n=n, st=st, tb=tb):
                    tau = 24 * n + 6 * k
                    for q, i in enumerate(reversed(range(6))):
                        if n == 0 and j in pre:
                            def f(i=i):
                                log.append(("r", ("pr", j, i), 0))
                                st["r1", j, i] = ws_b[zl + (PR + 2 * j), cb(i), LO]
                                st["r2", j, i] = ws_b[zl + (PR + 2 * j + 1), cb(i), LO]
                            at(tau - d_raw, 1, f)
                        else:
                            def f(i=i):
                                log.append(("r", ("t", n % 3, i), n))
                                v = ws[zl + (tb + j), cs(i), LO]
                                st["r1", j, i] = as_bf16(pltpu.roll(v, 1, 1))
                                st["r2", j, i] = as_bf16(pltpu.roll(v, 2, 1))
                            at(tau - d_rot + q, 1, f)
                        if n == NT - 1 and j in pre:
                            def f(i=i):
                                log.append(("r", ("t", 0, i), NT))
                                v = ws[zl + (TR + j), cs(i), LO]
                                st["q1", j, i] = pltpu.roll(v, 1, 1)
                                st["q2", j, i] = pltpu.roll(v, 2, 1)
                            at(24 + tau - d_rot + q, 1, f)
                            def f(i=i):
                                log.append(("w", ("pr", j, i), NT))
                                ws[zs + (PR + 2 * j), cs(i), LO] = st["q1", j, i]
                                ws[zs + (PR + 2 * j + 1), cs(i), LO] = st["q2", j, i]
                            at(24 + tau - d_rot + q + d_fix, 0, f)
                    def f():
                        for i in range(4): log.append(("r", ("t", n % 3, i), n))
                        st["r0", j] = ws_b[zl + (tb + j), 0:64, LO]
                    at(tau - d_raw + 1, 1, f)
                    for i in range(6):
                        def f(i=i):
                            st["l", j, i] = jnp.concatenate([ws_b[zl + (US + 2 * j), cb(i), LO], ws_b[zl + (US + 2 * j + 1), cb(i), LO]], axis=1)
                        at(tau - d_lhs + i, 1, f)
                    def f():
                        rhs = jnp.concatenate([st["r0", j][0:32]] + [st["r1", j, i] for i in range(6)] + [st["r0", j][32:64]] + [st["r2", j, i] for i in range(6)], axis=0)
                        lhs = jnp.concatenate([st["l", j, i] for i in range(6)], axis=0)
                        st["m", j] = mm(lhs, rhs)
                    at(tau, -1, f)
                def sched_rem(p, k, n=n, st=st, tb=tb):
                    tau = 24 * n + 6 * k
                    def f():
                        for i in (4, 5): log.append(("r", ("t", n % 3, i), n))
                        st["raw", p] = jnp.concatenate([ws_b[zl + (tb + 6 + q // 3), pl.ds(32 * (q % 3), 32), LO] for q in range(2 * p, 2 * p + 4)], axis=0)
                    at(tau - d_raw, 1, f)
                    for e in range(2):
                        for i in range(6):
                            def f(i=i, e=e):
                                st["lr", p, e, i] = ws_b[zl + (US + 12 + e), cb(i), LO]
                            at(tau - d_lhs + i, 1, f)
                        def f(e=e):
                            lhs = jnp.concatenate([st["lr", p, e, i] for i in range(6)], axis=0)
                            st["rm", p, e] = mm(lhs, st["raw", p])
                        at(tau, -1, f)
                sched_main(1, 0); sched_main(2, 0)
                sched_main(3, 1); sched_main(4, 1)
                sched_main(0, 2); sched_rem(0, 2)
                sched_main(5, 3); sched_rem(1, 3)
                def put(k, i, y, n=n):
                    log.append(("w", ("y", n, k, i), 1))
                    st16(zs + (YS + 4 * n + k), cb(i), y)
                for i in range(6):
                    rs = slice(16 * i, 16 * i + 16)
                    pr, po = PS + i // 3, pl.ds(16 * (i % 3), 16)
                    def f(i=i, rs=rs, st=st):
                        m1, m2 = st["m", 1][rs], st["m", 2][rs]
                        st["s", i] = m1 + m2
                        st["t", i] = m1 - m2
                        if pace and i % pace == pace - 1: ws[zs + PC, cs(i), LO] = as_u32(m1[0:8])
                    at(t0 + i, 0, f)
                    def f(i=i, rs=rs, st=st, pr=pr, po=po):
                        m3, m4 = st["m", 3][rs], st["m", 4][rs]
                        s, t = st["s", i], st["t", i]
                        u = m3 + m4
                        v = m3 - m4
                        zz = s + u
                        st["p0", i] = zz + s
                        st["p1", i] = B * (t + v)
                        ws[zs + pr, po, LO] = as_u32(zz + u)
                        ws[zs + (pr + 2), po, LO] = as_u32(A * (t + 4.0 * v))
                    at(t0 + 6 + i, 0, f)
                    def f(i=i, rs=rs, st=st, put=put):
                        put(0, i, (st["p0", i] + st["rm", 0, 0][rs]) + st["m", 0][rs])
                        put(1, i, st["p1", i] + st["rm", 0, 1][rs])
                    at(t0 + 12 + i, 0, f)
                    def f(i=i, st=st, pr=pr, po=po):
                        st["p2", i] = as_f32(ws[zl + pr, po, LO])
                        st["p3", i] = as_f32(ws[zl + (pr + 2), po, LO])
                    at(t0 + 18 + i - d_p, 1, f)
                    def f(i=i, rs=rs, st=st, put=put):
                        put(2, i, st["p2", i] + st["rm", 1, 0][rs])
                        put(3, i, (st["p3", i] + st["rm", 1, 1][rs]) + st["m", 5][rs])
                    at(t0 + 18 + i, 0, f)
                for q, i in enumerate(reversed(range(6))):
                    def f(i=i, n=n, st=st):
                        d, owner = tile_inputs(n + 2, i, hl, gmin)
                        for key in set(owner) - {None}:
                            if key[1] == 2:
                                for r in range(4 * key[0], 4 * key[0] + 6): log.append(("r", ("R", r, i), 1))
                        st["ts", i] = d, transform(d)
                    at(t0 + tf0 + int(tfs * q), 1, f)
                    def f(i=i, n=n, st=st):
                        log.append(("w", ("t", (n + 2) % 3, i), n + 2))
                        store_tile(n + 2, i, *st["ts", i], zs)
                    at(t0 + tf0 + int(tfs * q) + d_tf, 0, f)
            st = {}
            for g in range(2, 2 + NGRP):
                if rpos[g - 2] >= 24 * first:
                    for k in range(4):
                        for i in range(6):
                            r = 4 * g + 2 + k
                            p = rpos[g - 2] + (k * 6 + i) // 2
                            def f(i=i, r=r):
                                st["R", r, i] = pltpu.roll(ws[hl + (XS + r), cs(i), LO], 96, 1)
                            at(p, 1, f)
                            def f(i=i, r=r):
                                log.append(("w", ("R", r, i), 1))
                                ws[hs + (RS + r), cs(i), LO] = st["R", r, i]
                            at(p + d_fix, 0, f)
            for g in range(-1, NGRP - 1):
                if g >= gmin:
                    for k in range(4):
                        for i in range(6):
                            def f(g=g, k=k, i=i):
                                lo, hi, st["wrap", g, k, i], used = assemble_load(g % NGRP, k, i, zl)
                                for n in used: log.append(("r", ("y", n, k, i), 0 if g < 0 else 1))
                                ob[h0 + (4 * g + k), cs(i), LO] = lo
                                ob[h0 + (4 * g + k), cs(i), HI] = hi
                            p = apos[g + 1] + 6 * (k // 2) + i
                            at(p, 1, f)
                            def f(g=g, k=k, i=i):
                                v = st["wrap", g, k, i]
                                ob[h0 + (4 * g + k), cs(i), 0:v.shape[1]] = v
                            at(p + d_fix, 0, f)
                    if write is not None and g + 1 in wset:
                        at(apos[g + 1] + 11 + d_fix, 0.5, functools.partial(write, g))
            acts.sort(key=lambda a: a[:4])
            for a in acts:
                a[4]()
            cur = {}
            for i in range(6):
                for n in (first, first + 1): cur["t", n % 3, i] = n
                for j in pre: cur["pr", j, i] = 0
                for r in range(10 if first == 0 else 22): cur["R", r, i] = 1
                for n in range(NT):
                    for k in range(4): cur["y", n, k, i] = 0
            for op, key, ver in log:
                if op == "w": cur[key] = ver
                else: assert cur.get(key) == ver, (key, ver, cur.get(key))

        def body(hbase, rsem, writes, it, c):
            h0 = hbase + it * rows_it
            if rsem is not None:
                if wdyn:
                    @pl.when(it < nit - 1)
                    def _(): wait(rd(0, h0 + 10, rows_it, rsem.at[it]))
                    @pl.when(it == nit - 1)
                    def _(): wait(rd(0, h0 + 10, rows_it - 10, rsem.at[it]))
                else:
                    wait(rd(0, h0 + 10, rows_it, rsem.at[it]))
            def write(g):
                q = wset.index(g + 1)
                ng = (wset[q] - wset[q - 1] - 1) % NGRP + 1
                he = h0 + 4 * (g + 1)
                if wdyn:
                    c0 = it * len(wset) + q
                    lo = jnp.where(he - 4 * ng >= wdyn, he - 4 * ng, c0)
                    hi = jnp.where(he >= wdyn, he, c0 + 1)
                    start(wr(lo, hi - lo))
                else:
                    start(wr(he - 4 * ng, 4 * ng), q % 2 if wprio else 0)
            run(0, -1, h0, z_ref[0], z_ref[1], write if writes else None)
            return c

        def main(rsem, fsem):
            wcp = [pltpu.make_async_copy(w_hbm, w_ref, fsem.at[0])]
            first = rd(H - 2, 0, 2, fsem.at[1]) + rd(0, 2, 4, fsem.at[1])
            second = rd(4, 6, 8, fsem.at[2])
            if wfirst:
                start(wcp); start(first)
            else:
                start(first); start(wcp)
            start(second)
            for i in range(nr):
                d = 14 + i * rows_it
                start(rd(d - 2, d, min(rows_it, H - d), rsem.at[i]))
            if not wdyn:
                d = 14 + n1 * rows_it
                rest = rd(d - 2, d, H - d, fsem.at[3])
                start(rest)
            z_ref[0] = 0
            z_ref[1] = 0
            for r in range(H + 2, XR):
                ws[XS + r] = jnp.zeros((C // 2, W), U32)
            def prime():
                for h in range(6):
                    ws[RS + h, :, LO] = pltpu.roll(ws[XS + h, :, LO], 96, 1)
                for h in range(2):
                    ws[XS + H + h] = ws[XS + h]
                for n in (NT - 2, NT - 1):
                    for i in range(6):
                        d, _ = tile_inputs(n, i, 4 - rows_it, NGRP - 1)
                        store_tile(n, i, d, transform(d), 0)
            if wfirst:
                wait(wcp); weights(); wait(first); prime()
            else:
                wait(first); prime(); wait(wcp); weights()
            wait(second)
            run(NT - 2, NGRP - 1, 4 - rows_it, z_ref[0], z_ref[1], None)
            assert wset[-1] == NGRP - 1
            if wdyn:
                lax.fori_loop(0, nit, functools.partial(body, 4, rsem, True), 0)
            else:
                lax.fori_loop(0, n1, functools.partial(body, 4, rsem, False), 0)
                start(wr(0, n1 * rows_it))
                wait(rest)
                lax.fori_loop(0, nit - n1, functools.partial(body, 4 + n1 * rows_it, None, True), 0)
            for k in range(4):
                for i in range(6):
                    lo, hi, wrap, _ = assemble_load(NGRP - 1, k, i, 0)
                    ob[H - 4 + k, cs(i), LO] = lo
                    ob[H - 4 + k, cs(i), HI] = hi
                    ob[H - 4 + k, cs(i), 0:wrap.shape[1]] = wrap
            start(wr(H - 4, 4))
        pl.run_scoped(main, pltpu.SemaphoreType.DMA((nr,)), pltpu.SemaphoreType.DMA((4,)))
        wait(wr(0, H))

    @jax.jit
    def fn(x, w):
        xt = x.transpose(0, 1, 3, 2).reshape(H, C, W)
        o = pl.pallas_call(
            kernel,
            in_specs=[pl.BlockSpec(memory_space=pl.ANY), pl.BlockSpec(memory_space=pl.ANY)],
            out_specs=pl.BlockSpec(memory_space=pl.ANY),
            out_shape=jax.ShapeDtypeStruct((H, C, W), BF16),
            scratch_shapes=[
                pltpu.VMEM((NROWS, C // 2, W), U32), pltpu.VMEM((H, C // 2, W), U32),
                pltpu.VMEM((3, 3, C, C), BF16),
                pltpu.SMEM((2,), jnp.int32),
                pltpu.SemaphoreType.DMA((1,)),
            ],
            compiler_params=pltpu.CompilerParams(vmem_limit_bytes=100 * 2 ** 20, flags=flags),
        )(xt, w)
        return o.reshape(1, H, C, W).transpose(0, 1, 3, 2)
    return fn


pallas_standalone__fft_conv__vision_kernel = make()
```

```python
import functools

import jax
import jax.numpy as jnp
import numpy as np
from jax import lax
from jax.experimental import pallas as pl
from jax.experimental.pallas import tpu as pltpu

H = W = 224
C = 96
LANES = 128
F32, BF16, U32 = jnp.float32, jnp.bfloat16, jnp.uint32

A, B = float(2.0**-0.5), float(2.0**0.5)


def _filter_transform():
    points = [0.0, A, -A, B, -B]
    g = np.zeros((6, 3))
    for j, p in enumerate(points):
        norm = np.prod([p - q for q in points if q != p])
        g[j] = [p**i / norm for i in range(3)]
    g[5, 2] = 1.0
    g[1:5] *= 0.5
    return np.round(g, 12)


G = _filter_transform()


def _input_transform(d):
    r = d[4] - d[2]
    e1, e2 = r - d[2], r + d[4]
    q = d[3] - d[1]
    o1, o2 = A * (q - d[1]), B * (q + d[3])
    return [(d[0] + d[4]) - 2.5 * d[2], e1 + o1, e1 - o1,
            e2 + o2, e2 - o2, (d[1] + d[5]) - 2.5 * d[3]]


PERIOD_GROUPS, PERIOD_TILES = 5, 9
NUM_GROUPS = H // 4


def _pack_period():
    tiles, pieces, room, start = [], [], LANES, 2
    for g in range(PERIOD_GROUPS):
        end = start + W
        while start < end:
            stop = min(end, start + room - 2)
            pieces.append((g, start, stop))
            room -= stop - start + 2
            start = stop
            if room == 0:
                tiles.append(pieces)
                pieces, room = [], LANES
        start = (start + 2) % LANES
    tiles.append(pieces)
    assert len(tiles) == PERIOD_TILES
    return tiles


PERIOD = _pack_period()
NUM_TILES = 2 + PERIOD_TILES * ((NUM_GROUPS - 1) // PERIOD_GROUPS)


def _pieces(n):
    p, m = divmod(n - 2, PERIOD_TILES)
    first = 1 + PERIOD_GROUPS * p
    return [(first + g, a, b) for g, a, b in PERIOD[m] if first + g >= 0]


def _merge(owner, load):
    last = next(k for k in owner if k is not None)
    runs = []
    for lane, k in enumerate(owner):
        last = last if k is None else k
        if not runs or runs[-1][0] != last:
            runs.append([last, lane, lane])
        runs[-1][2] = lane + 1
    vals = {}
    for k, _, _ in runs:
        if k not in vals:
            vals[k] = load(k)
    if len(runs) == 3 and runs[0][0] == runs[2][0]:
        lane = lax.broadcasted_iota(jnp.int32, (8, LANES), 1)
        inside = (lane >= runs[1][1]) & (lane < runs[1][2])
        return jnp.where(inside, vals[runs[1][0]], vals[runs[0][0]])
    return jnp.concatenate([vals[k][:, a:b] for k, a, b in runs], axis=1)


X_SLABS = H + 10
X_WRAP = X_SLABS
X_FENCE_LO = 2 * X_SLABS
X_FENCE_HI = X_SLABS
X_FILTER = X_SLABS + 1
T_ROLLED = 3 * 8
T_FENCE = T_ROLLED + 12
V_FILTER = 4 * PERIOD_TILES
V_FENCE = V_FILTER + 14
O_PARTIAL = H
STEPS = 24


def _as_bf16(v):
    return pltpu.bitcast(v, BF16)


def _as_u32(v):
    return pltpu.bitcast(v, U32)


def _words(i):
    return pl.ds(8 * i, 8)


def _chans(i):
    return pl.ds(16 * i, 16)


def _slab(zero, s, rows):
    return zero + s // 2, rows, pl.ds(LANES * (s % 2), LANES)


def _store_bf16(ref, zero, s, rows, value):
    lead, rows, lanes = _slab(zero, s, rows)
    ref[pl.ds(lead, 1), rows, lanes] = value[None].astype(BF16)


def make(BLOCKS=((3, 1), (6, 1), (11, 1), (12, 1), (15, 1), (27, 2)),
         LEAD_LHS=11, LEAD_ROLL=27, LEAD_RAW=13, LEAD_PLAIN=15, LEAD_PARTIAL=2, ROLL_DELAY=10, TRANSFORM_DELAY=3,
         TRANSFORM_AT=(0, 4, 8, 12, 16, 18), WRAP_AT=(-48, -22, 26, 74, 122), WRAP_LEN=(14, 14, 14, 16, 14),
         GATHER_AT=(40, 88, 136, 182, 205), GATHER_LEN=(7, 5, 7, 7, 6), DMA_AT=13,
         BULK_READS=3, READ_TILE=7, READ_BURST=14, READS_PER_PERIOD=36, WRITE_TILE=47, WRITES_PER_PERIOD=34,
         WGAP=14, WDEPTH=3, RDIST=8, scopes=False, flags=None):
    PRE_ROLLED = (1, 2, 3, 4)
    ENDS = np.cumsum([n for n, reps in BLOCKS for _ in range(reps)]).tolist()
    assert ENDS[-1] == NUM_TILES

    def _wrap_step(g):
        p, m = divmod(g - 1, PERIOD_GROUPS)
        return STEPS * (2 + PERIOD_TILES * p) + WRAP_AT[m]

    def _gather_step(row, i):
        p, m = divmod(row // 4 - 1, PERIOD_GROUPS)
        step = STEPS * (2 + PERIOD_TILES * p) + GATHER_AT[m] + 6 * (row % 4 // 2)
        for end in ENDS:
            if step < STEPS * end < step + GATHER_LEN[m] + ROLL_DELAY - 5:
                step = STEPS * end
        return step + (2 * i + row % 2) * GATHER_LEN[m] // 12

    def _slabs_needed(end):
        g = max(g for g, _, _ in _pieces(end + 1))
        while _wrap_step(g + 1) < STEPS * end:
            g += 1
        return min(4 * g + 6, H)

    def _plan_reads():
        edges = [6] + [_slabs_needed(end) for end in ENDS]
        order = []
        for block in range(BULK_READS, len(ENDS)):
            s = edges[block]
            while s < edges[block + 1]:
                d = min(RDIST, (edges[block + 1] - s) // 2)
                order += [(s + i + e * d, block) for i in range(d) for e in range(2)]
                s += 2 * d
        tiles = [READ_TILE] * READ_BURST + [
            READ_TILE + 1 + PERIOD_TILES * q // READS_PER_PERIOD
            for q in range(len(order) - READ_BURST)]
        assert all(t < ENDS[block - 1] for t, (_, block) in zip(tiles, order))
        return edges, [(t,) + o for t, o in zip(tiles, order)]

    def _plan_writes():
        count = (NUM_TILES - WRITE_TILE) * WRITES_PER_PERIOD // PERIOD_TILES
        tiles = [NUM_TILES - 1 - PERIOD_TILES * q // WRITES_PER_PERIOD
                 for q in reversed(range(count))]
        left, order = list(range(H - 4)), []
        for step in ([STEPS * WRITE_TILE] * (H - 4 - count)
                     + [STEPS * t + DMA_AT for t in tiles]):
            ready = [r for r in left if _gather_step(r, 5) + ROLL_DELAY < step]
            for depth in range(WDEPTH, -1, -1):
                far = [r for r in ready if all(
                    abs(r - q) >= WGAP for q in order[len(order) - depth:])]
                if far:
                    break
            order.append(far[-1])
            left.remove(far[-1])
        return order[:H - 4 - count], list(zip(tiles, order[H - 4 - count:]))

    READ_EDGES, READS = _plan_reads()
    WRITE_BURST, WRITES = _plan_writes()
    S_READS, S_WRITES = 2, 2 + len(READS)

    def _kernel(x_hbm, w_hbm, o_hbm, x_lo16, x_hi16, o_lo16, o_hi16, t_buf, v_buf,
                scalars, write_sem):
        x_lo, x_hi, o_lo, o_hi = [
            r.bitcast(U32) for r in (x_lo16, x_hi16, o_lo16, o_hi16)]
        t_buf16, v_buf16 = t_buf.bitcast(BF16), v_buf.bitcast(BF16)
        lo, hi = pl.ds(0, LANES), pl.ds(LANES, W - LANES)

        def read(row, slab, n, sem):
            return [pltpu.make_async_copy(
                x_hbm.at[pl.ds(row, n), :, cols], buf.at[pl.ds(slab, n)], sem)
                for cols, buf in ((lo, x_lo16), (hi, x_hi16))]

        def write(row, n):
            return [pltpu.make_async_copy(
                buf.at[pl.ds(row, n)], o_hbm.at[pl.ds(row, n), :, cols], write_sem)
                for cols, buf in ((lo, o_lo16), (hi, o_hi16))]

        def start(copies, priority=0):
            for c in copies:
                c.start(priority=priority)

        nw = [0]

        def wait(copies):
            if scopes:
                nw[0] += 1
                with jax.named_scope("wait%02d" % nw[0]):
                    for c in copies:
                        c.wait()
                return
            for c in copies:
                c.wait()

        def transform_filter():
            eye = (lax.broadcasted_iota(jnp.int32, (C, C), 0)
                   == lax.broadcasted_iota(jnp.int32, (C, C), 1)).astype(BF16)

            def transposed(parts):
                return lax.dot_general(
                    eye, jnp.concatenate(parts, axis=0), (((1,), (1,)), ((), ())),
                    preferred_element_type=F32)

            def tap(i, kw, rows=slice(None)):
                return x_hi16[X_FILTER + 3 * (2 - i) + kw, rows, :]

            for e in range(2):
                f = [transposed([tap(i, 0, pl.ds(32 * e, 32)), tap(i, 1 + e)])
                     for i in range(3)]
                for j in range(6):
                    u = functools.reduce(jnp.add, [
                        f[i] * float(G[j, i]) for i in (0, 2, 1) if G[j, i] != 0.0])
                    _store_bf16(v_buf16, 0, V_FILTER + 2 * j + e, slice(None), u)
            direct = [tap(i, 0, pl.ds(64, 32)) for i in range(3)]
            pad = [jnp.zeros((32, C), BF16)]
            _store_bf16(v_buf16, 0, V_FILTER + 12, slice(None), transposed(direct + pad))
            _store_bf16(v_buf16, 0, V_FILTER + 13, slice(None), transposed(pad + direct))

        def transform_tile(n, i, row0):
            owner = [None] * LANES
            for g, a, b in _pieces(n):
                for c in range(a - 2, b):
                    owner[c % LANES] = (LANES <= c < W, 4 * g + (X_WRAP if c >= W else 0))

            def load(q, key):
                return (x_hi if key[0] else x_lo)[row0 + (key[1] + q), _words(i), :]

            d = [_merge(owner, functools.partial(load, q)) for q in range(6)]
            t = _input_transform([_as_bf16(v).astype(F32) for v in d])

            def store(zero):
                base = 8 * (n % 3)
                for j in range(6):
                    _store_bf16(t_buf16, zero, base + j, _chans(i), t[j])
                if i >= 4:
                    for q in range(6):
                        rows = _words(2 * (q % 3) + i - 4)
                        t_buf[_slab(zero, base + 6 + q // 3, rows)] = d[q]
            return store

        def gather_row(row, i, zero, row0):
            low, wrapped, high = [None] * LANES, [None] * LANES, None
            for n in range(NUM_TILES):
                for g, a, b in _pieces(n):
                    for c in range(a, b) if g == row // 4 else ():
                        if c < LANES:
                            low[c] = n
                        elif c < W:
                            assert high in (None, n)
                            high = n
                        else:
                            wrapped[c % LANES] = n
            loaded = {}

            def load(n):
                if n not in loaded:
                    s = 4 * (n % PERIOD_TILES) + row % 4
                    loaded[n] = v_buf[_slab(zero, s, _words(i))]
                return loaded[n]

            rolled = pltpu.roll(_merge(wrapped, load), 2 * LANES - W, 1)
            o_lo[row0 + row, _words(i), :] = _merge(low, load)
            o_hi[row0 + row, _words(i), :] = load(high)[:, :W - LANES]
            width = low.count(None)

            def store():
                o_lo[row0 + row, _words(i), :width] = rolled[:, :width]
            return store

        def run_block(first, end, rep, read_sems, zl, zs):
            periods = rep * ((end - first) // PERIOD_TILES)
            row_l = periods * (4 * PERIOD_GROUPS) + zl
            row_s = periods * (4 * PERIOD_GROUPS) + zs
            work, val = [], {}
            DOT, STORE, COPY, LOAD = range(4)

            def at(step, kind, *args):
                def register(fn):
                    rel = min(step, STEPS * end) - STEPS * first
                    key = (rel, kind, 0) if rel >= 0 else (-1, 0, rel)
                    work.append((key, len(work), functools.partial(fn, *args)))
                return register

            def fence(step, v, stored):
                v, rows = _as_u32(v[:8]), _words(step % 6)
                if step % 2 == 0:
                    t_buf[_slab(zs, T_FENCE, rows)] = v
                    x_lo[zs + X_FENCE_LO, rows, :] = v
                elif not stored:
                    v_buf[_slab(zs, V_FENCE, rows)] = v
                if (step + 1) % STEPS in TRANSFORM_AT:
                    x_hi[zs + X_FENCE_HI, rows, :] = v[:, :W - LANES]

            def filter_rows(name, step, slabs):
                for i in range(6):
                    @at(step - LEAD_LHS + i, LOAD, i)
                    def _(i):
                        val[name, i] = jnp.concatenate(
                            [v_buf16[_slab(zl, s, _chans(i))] for s in slabs], axis=1)
                return lambda: jnp.concatenate(
                    [val.pop((name, i)) for i in range(6)], axis=0)

            def product(n, j, step):
                src = 8 * (n % 3) + j
                for q, i in enumerate(reversed(range(6))):
                    if n == first and j in PRE_ROLLED:
                        @at(step - LEAD_RAW, LOAD, i)
                        def _(i):
                            val["rolled", n, j, i] = [
                                t_buf16[_slab(zl, T_ROLLED + 2 * j + e, _chans(i))]
                                for e in range(2)]
                    else:
                        @at(step - LEAD_ROLL + q, LOAD, i)
                        def _(i):
                            v = t_buf[_slab(zl, src, _words(i))]
                            val["rolled", n, j, i] = [
                                _as_bf16(pltpu.roll(v, 1 + e, 1)) for e in range(2)]
                    if n == end - 1 and j in PRE_ROLLED:
                        @at(step + STEPS - LEAD_ROLL + q, LOAD, i)
                        def _(i):
                            v = t_buf[_slab(zl, 8 * (end % 3) + j, _words(i))]
                            val["next", j, i] = [
                                pltpu.roll(v, 1 + e, 1) for e in range(2)]

                        @at(step + STEPS - LEAD_ROLL + q + ROLL_DELAY, STORE, i)
                        def _(i):
                            for e, v in enumerate(val["next", j, i]):
                                t_buf[_slab(zs, T_ROLLED + 2 * j + e, _words(i))] = v

                @at(step - LEAD_PLAIN, LOAD)
                def _():
                    val["plain", n, j] = t_buf16[_slab(zl, src, pl.ds(0, 64))]

                lhs = filter_rows(
                    ("u", n, j), step, [V_FILTER + 2 * j + e for e in range(2)])

                @at(step, DOT)
                def _():
                    rhs = []
                    for e in range(2):
                        rhs.append(val["plain", n, j][32 * e:32 * e + 32])
                        rhs += [val["rolled", n, j, i][e] for i in range(6)]
                    val["m", n, j] = jnp.dot(
                        lhs(), jnp.concatenate(rhs, axis=0), preferred_element_type=F32)

            def direct(n, k, step):
                @at(step - LEAD_RAW, LOAD)
                def _():
                    val["raw", n, k] = jnp.concatenate([
                        t_buf16[_slab(zl, 8 * (n % 3) + 6 + q // 3, pl.ds(32 * (q % 3), 32))]
                        for q in range(k, k + 4)], axis=0)

                for e in range(2):
                    lhs = filter_rows(("r", n, k + e), step, [V_FILTER + 12 + e])

                    @at(step, DOT, e, lhs)
                    def _(e, lhs):
                        val["d", n, k + e] = jnp.dot(
                            lhs(), val["raw", n, k], preferred_element_type=F32)

            def output_transform(n, i):
                t0 = STEPS * n
                partial = [(O_PARTIAL + 2 * e + i // 3, pl.ds(16 * (i % 3), 16))
                           for e in range(2)]

                def result(kind, j):
                    return val[kind, n, j][16 * i:16 * i + 16]

                def put(k, y):
                    _store_bf16(v_buf16, zs, 4 * (n % PERIOD_TILES) + k, _chans(i), y)

                @at(t0 + i, STORE)
                def _():
                    m1, m2 = result("m", 1), result("m", 2)
                    val["st", n, i] = m1 + m2, m1 - m2
                    fence(i, m1, False)

                @at(t0 + 6 + i, STORE)
                def _():
                    m3, m4 = result("m", 3), result("m", 4)
                    s, t = val["st", n, i]
                    u, v = m3 + m4, m3 - m4
                    z = s + u
                    val["p01", n, i] = z + s, B * (t + v)
                    o_lo[zs + partial[0][0], partial[0][1], :] = _as_u32(z + u)
                    fence(6 + i, m3, False)
                    o_lo[zs + partial[1][0], partial[1][1], :] = _as_u32(A * (t + 4.0 * v))

                @at(t0 + 12 + i, STORE)
                def _():
                    p0, p1 = val["p01", n, i]
                    put(0, (p0 + result("d", 0)) + result("m", 0))
                    y1 = p1 + result("d", 1)
                    put(1, y1)
                    fence(12 + i, y1, True)

                @at(t0 + 18 + i - LEAD_PARTIAL, LOAD)
                def _():
                    val["p23", n, i] = [
                        pltpu.bitcast(o_lo[zl + s, rows, :], F32) for s, rows in partial]

                @at(t0 + 18 + i, STORE)
                def _():
                    p2, p3 = val["p23", n, i]
                    y2 = p2 + result("d", 2)
                    put(2, y2)
                    fence(18 + i, y2, True)
                    put(3, (p3 + result("d", 3)) + result("m", 5))

            for n in range(first, end):
                t0 = STEPS * n
                product(n, 1, t0)
                product(n, 2, t0)
                product(n, 3, t0 + 6)
                product(n, 4, t0 + 6)
                product(n, 0, t0 + 12)
                direct(n, 0, t0 + 12)
                product(n, 5, t0 + 18)
                direct(n, 2, t0 + 18)
                for i in range(6):
                    output_transform(n, i)
                for step, i in zip(TRANSFORM_AT, reversed(range(6))):
                    @at(t0 + step, LOAD, n, i)
                    def _(n, i):
                        val["t", n, i] = transform_tile(n + 2, i, row_l)

                    @at(t0 + step + TRANSFORM_DELAY, STORE, n, i)
                    def _(n, i):
                        val["t", n, i](zs)

            for g in range(1, NUM_GROUPS + 2):
                if STEPS * first <= _wrap_step(g) < STEPS * end:
                    length = WRAP_LEN[(g - 1) % PERIOD_GROUPS]
                    for k in range(4):
                        for i in range(6):
                            step = _wrap_step(g) + ((5 - i) * 4 + k) * length // 24

                            @at(step, LOAD, 4 * g + 2 + k, i)
                            def _(s, i):
                                val["wrap", s, i] = pltpu.roll(
                                    x_lo[row_l + s, _words(i), :], W - LANES, 1)

                            @at(step + ROLL_DELAY, STORE, 4 * g + 2 + k, i)
                            def _(s, i):
                                x_lo[row_s + (X_WRAP + s), _words(i), :] = val["wrap", s, i]

            for row in range(H):
                if STEPS * first <= _gather_step(row - row % 2, 0) < STEPS * end:
                    for i in range(6):
                        @at(_gather_step(row, i), LOAD, row, i)
                        def _(row, i):
                            val["y", row, i] = gather_row(row, i, zl, row_s)

                        @at(_gather_step(row, i) + ROLL_DELAY, STORE, row, i)
                        def _(row, i):
                            val["y", row, i]()

            for q, (n, s, block) in enumerate(READS):
                if first <= n < end:
                    @at(STEPS * n + DMA_AT, COPY, q, s, block)
                    def _(q, s, block):
                        if not isinstance(rep, int):
                            v = scalars[periods * READS_PER_PERIOD + (S_READS + q)]
                            s, block = v & 255, v >> 8
                        start(read(s - 2, s, 1, read_sems.at[block]), q % 2)

            if isinstance(rep, int) and first <= WRITE_TILE < end:
                @at(STEPS * WRITE_TILE, COPY)
                def _():
                    for row in WRITE_BURST:
                        start(write(row, 1))

            for q, (n, row) in enumerate(WRITES):
                if first <= n < end:
                    @at(STEPS * n + DMA_AT, COPY, q, row)
                    def _(q, row):
                        if not isinstance(rep, int):
                            row = scalars[periods * WRITES_PER_PERIOD + (S_WRITES + q)]
                        start(write(row, 1))

            for _, _, fn in sorted(work, key=lambda item: item[:2]):
                fn()

        def compute(read_sems, first_sems):
            def block_rows(block):
                s, n = READ_EDGES[block], READ_EDGES[block + 1] - READ_EDGES[block]
                return read(s - 2, s, n, read_sems.at[block])

            first_rows = (read(H - 2, 0, 2, first_sems.at[0])
                          + read(0, 2, 4, first_sems.at[0]))
            taps = [pltpu.make_async_copy(
                w_hbm, x_hi16.at[pl.ds(X_FILTER, 9)], first_sems.at[1])]
            start(first_rows + taps)
            for block in range(BULK_READS):
                start(block_rows(block))
            scalars[0] = 0
            scalars[1] = 0
            for q, (_, s, block) in enumerate(READS):
                scalars[S_READS + q] = s + 256 * block
            for q, (_, row) in enumerate(WRITES):
                scalars[S_WRITES + q] = row
            for s in range(H + 2, X_SLABS):
                x_lo[s] = jnp.zeros(x_lo.shape[1:], U32)
                x_hi[s] = jnp.zeros(x_hi.shape[1:], U32)

            wait(first_rows)
            for s in range(6):
                x_lo[X_WRAP + s] = pltpu.roll(x_lo[s], W - LANES, 1)
            for s in range(2):
                x_lo[H + s] = x_lo[s]
                x_hi[H + s] = x_hi[s]
            for n in range(2):
                for i in range(6):
                    transform_tile(n, i, 0)(0)
            wait(taps)
            for j in PRE_ROLLED:
                for e in range(2):
                    t_buf[_slab(0, T_ROLLED + 2 * j + e, slice(None))] = pltpu.roll(
                        t_buf[_slab(0, j, slice(None))], 1 + e, 1)
            transform_filter()

            zl, zs = scalars[0], scalars[1]
            block = first = 0
            for tiles, reps in BLOCKS:
                if reps == 1:
                    wait(block_rows(block))
                    run_block(first, first + tiles, 0, read_sems, zl, zs)
                else:
                    if first == WRITE_TILE:
                        for row in WRITE_BURST:
                            start(write(row, 1))

                    @pl.loop(0, reps)
                    def _(rep):
                        for i in range(reps):
                            pl.when(rep == i)(lambda: wait(block_rows(block + i)))
                        run_block(first, first + tiles, rep, read_sems, zl, zs)
                block += reps
                first += tiles * reps

            assert _gather_step(H - 3, 0) < STEPS * NUM_TILES <= _gather_step(H - 2, 0)
            start(write(H - 4, 2))
            stores = [gather_row(row, i, 0, 0) for row in (H - 2, H - 1) for i in range(6)]
            last_lo, last_hi = write(H - 2, 2)
            last_hi.start()
            for store in stores:
                store()
            last_lo.start()

        pl.run_scoped(compute, pltpu.SemaphoreType.DMA((len(ENDS),)),
                      pltpu.SemaphoreType.DMA((2,)))
        wait(write(0, H))

    @jax.jit
    def fn(x, w):
        assert x.shape == (1, H, W, C) and w.shape == (3, 3, C, C)
        y = pl.pallas_call(
            _kernel,
            in_specs=[pl.BlockSpec(memory_space=pl.ANY)] * 2,
            out_specs=pl.BlockSpec(memory_space=pl.ANY),
            out_shape=jax.ShapeDtypeStruct((H, C, W), BF16),
            scratch_shapes=[
                pltpu.VMEM((2 * X_SLABS + 2, C, LANES), BF16),
                pltpu.VMEM((X_SLABS + 10, C, W - LANES), BF16),
                pltpu.VMEM((H + 4, C, LANES), BF16),
                pltpu.VMEM((H, C, W - LANES), BF16),
                pltpu.VMEM((T_FENCE // 2 + 1, C // 2, 2 * LANES), U32),
                pltpu.VMEM((V_FENCE // 2 + 1, C // 2, 2 * LANES), U32),
                pltpu.SMEM((S_WRITES + len(WRITES),), jnp.int32),
                pltpu.SemaphoreType.DMA(()),
            ],
            compiler_params=pltpu.CompilerParams(
                vmem_limit_bytes=64 * 2**20, disable_bounds_checks=True, flags=flags),
        )(x.transpose(0, 1, 3, 2).reshape(H, C, W), w.reshape(9, C, C))
        return y.reshape(1, H, C, W).transpose(0, 1, 3, 2)
    return fn


pallas_standalone__fft_conv__vision_kernel = make()
```

```python
import functools

import jax
import jax.numpy as jnp
import numpy as np
from jax import lax
from jax.experimental import pallas as pl
from jax.experimental.pallas import tpu as pltpu

H = W = 224
C = 96
LANES = 128
F32, BF16, U32 = jnp.float32, jnp.bfloat16, jnp.uint32

A, B = float(2.0**-0.5), float(2.0**0.5)


def _filter_transform():
    points = [0.0, A, -A, B, -B]
    g = np.zeros((6, 3))
    for j, p in enumerate(points):
        norm = np.prod([p - q for q in points if q != p])
        g[j] = [p**i / norm for i in range(3)]
    g[5, 2] = 1.0
    g[1:5] *= 0.5
    return np.round(g, 12)


G = _filter_transform()


def _input_transform(d):
    r = d[4] - d[2]
    e1, e2 = r - d[2], r + d[4]
    q = d[3] - d[1]
    o1, o2 = A * (q - d[1]), B * (q + d[3])
    return [(d[0] + d[4]) - 2.5 * d[2], e1 + o1, e1 - o1,
            e2 + o2, e2 - o2, (d[1] + d[5]) - 2.5 * d[3]]


PERIOD_GROUPS, PERIOD_TILES = 5, 9
NUM_GROUPS = H // 4


def _pack_period():
    tiles, pieces, room, start = [], [], LANES, 2
    for g in range(PERIOD_GROUPS):
        end = start + W
        while start < end:
            stop = min(end, start + room - 2)
            pieces.append((g, start, stop))
            room -= stop - start + 2
            start = stop
            if room == 0:
                tiles.append(pieces)
                pieces, room = [], LANES
        start = (start + 2) % LANES
    tiles.append(pieces)
    assert len(tiles) == PERIOD_TILES
    return [[(PERIOD_GROUPS - 1 - g, a, b) for g, a, b in t] for t in tiles[::-1]]


PERIOD = _pack_period()
NUM_TILES = 2 + PERIOD_TILES * ((NUM_GROUPS - 1) // PERIOD_GROUPS)


def _pieces(n):
    p, m = divmod(n - 2, PERIOD_TILES)
    first = 1 + PERIOD_GROUPS * p
    return [(first + g, a, b) for g, a, b in PERIOD[m] if first + g >= 0]


def _merge(owner, load):
    last = next(k for k in owner if k is not None)
    runs = []
    for lane, k in enumerate(owner):
        last = last if k is None else k
        if not runs or runs[-1][0] != last:
            runs.append([last, lane, lane])
        runs[-1][2] = lane + 1
    vals = {}
    for k, _, _ in runs:
        if k not in vals:
            vals[k] = load(k)
    if len(runs) == 3 and runs[0][0] == runs[2][0]:
        lane = lax.broadcasted_iota(jnp.int32, (8, LANES), 1)
        inside = (lane >= runs[1][1]) & (lane < runs[1][2])
        return lax.select(inside, vals[runs[1][0]], vals[runs[0][0]])
    return jnp.concatenate([vals[k][:, a:b] for k, a, b in runs], axis=1)


STEPS = 24
BLOCKS = ((2, 1), (4, 1), (9, 1), (14, 1), (18, 1), (27, 2))
ENDS = np.cumsum([n for n, reps in BLOCKS for _ in range(reps)]).tolist()
LEAD_FILTER, LEAD_ROLL, LEAD_RAW, LEAD_PLAIN, LEAD_PARTIAL = 11, 28, 13, 15, 4
ROLL_DELAY, TRANSFORM_DELAY = 10, 4
TRANSFORM_AT = (0, 4, 10, 12, 17, 18)
PRE_ROLLED = (1, 2, 3, 4)
WRAP_AT, WRAP_LEN = (-72, -46, 2, 50, 99), (20, 14, 14, 14, 14)
GATHER_AT, GATHER_LEN = (14, 64, 111, 158, 182), (7, 7, 7, 7, 4)
FINISH_AT = (38, 86, 134, 182, 206)
COPY_AT = 12
BULK_READS = 4
READ_TILE, READ_BURST, READS_PER_PERIOD = 11, 20, 36
WRITE_TILE, WRITES_PER_PERIOD = 47, 34
assert ENDS[-1] == NUM_TILES and WRITE_TILE == ENDS[-1 - BLOCKS[-1][1]]


def _group_step(g, table):
    p, m = divmod(g - 1, PERIOD_GROUPS)
    return STEPS * (2 + PERIOD_TILES * p) + table[m]


def _gather_step(row, i):
    step = _group_step(row // 4, GATHER_AT) + 6 * (row % 4 // 2)
    length = GATHER_LEN[(row // 4 - 1) % PERIOD_GROUPS]
    for end in ENDS:
        if step < STEPS * end < step + length + ROLL_DELAY - 5:
            step = STEPS * end
    return step + (2 * i + row % 2) * length // 12


def _finish_step(row, i):
    return _group_step(row // 4, FINISH_AT) + 6 * (row % 4 // 2) + i


def _plan_reads():
    low, high = [10], [6]
    for block, end in enumerate(ENDS):
        g = max(g for g, _, _ in _pieces(end + 1))
        while _group_step(g + 1, WRAP_AT) < STEPS * end:
            g += 1
        low.append(min(4 * g + 6, H))
        high.append(low[-1] if block >= BULK_READS - 1 else max(
            4 * g + 6 for n in range(end + 2) for g, a, b in _pieces(n)
            if b > LANES and a - 2 < W))
    order = []
    for block in range(BULK_READS, len(ENDS)):
        s = low[block]
        while s < low[block + 1]:
            d = min(8, (low[block + 1] - s) // 2)
            order += [(s + i + e * d, block) for i in range(d) for e in range(2)]
            s += 2 * d
    tiles = [READ_TILE] * READ_BURST + [
        READ_TILE + 1 + PERIOD_TILES * q // READS_PER_PERIOD
        for q in range(len(order) - READ_BURST)]
    assert all(t < min(ENDS[block - 1], WRITE_TILE)
               for t, (_, block) in zip(tiles, order))
    return (low, high), [(t,) + o for t, o in zip(tiles, order)]


def _plan_writes():
    count = (NUM_TILES - WRITE_TILE) // PERIOD_TILES * WRITES_PER_PERIOD
    tiles = [NUM_TILES - 1 - PERIOD_TILES * q // WRITES_PER_PERIOD
             for q in reversed(range(count))]
    left, order = list(range(H - 4)), []
    for step in ([STEPS * WRITE_TILE] * (H - 4 - count)
                 + [STEPS * t + COPY_AT for t in tiles]):
        ready = [r for r in left if _finish_step(r, 5) < step]
        for depth in (3, 2, 1, 0):
            recent = order[max(len(order) - depth, 0):]
            far = [r for r in ready if all(abs(r - q) >= 14 for q in recent)]
            if far:
                break
        order.append(far[-1])
        left.remove(far[-1])
    return order[:H - 4 - count], list(zip(tiles, order[H - 4 - count:]))


READ_EDGES, READS = _plan_reads()
FIRST_WRITES, WRITES = _plan_writes()

X_SLABS = H + 10
X_WRAP = X_SLABS
X_FENCE_LO = 2 * X_SLABS
X_FENCE_HI = X_SLABS
X_FILTER = X_SLABS + 1
T_ROLLED = 3 * 8
T_FENCE = T_ROLLED + 12
V_FILTER = 4 * PERIOD_TILES
V_FENCE = V_FILTER + 14
O_PARTIAL = H


def _as_bf16(v):
    return pltpu.bitcast(v, BF16)


def _as_u32(v):
    return pltpu.bitcast(v, U32)


def _words(i):
    return pl.ds(8 * i, 8)


def _chans(i):
    return pl.ds(16 * i, 16)


def _from(base):
    return functools.lru_cache(None)(lambda offset: base + offset)


def _slab(index, s, rows):
    return index(s // 2), rows, pl.ds(LANES * (s % 2), LANES)


def _store_bf16(ref, index, s, rows, value):
    lead, rows, lanes = _slab(index, s, rows)
    ref[pl.ds(lead, 1), rows, lanes] = value[None].astype(BF16)


def _kernel(x_hbm, w_hbm, o_hbm, x_lo16, x_hi16, o_lo16, o_hi16, t_buf, v_buf,
            scalars, write_sem):
    x_lo, x_hi, o_lo, o_hi = [
        r.bitcast(U32) for r in (x_lo16, x_hi16, o_lo16, o_hi16)]
    t_buf16, v_buf16 = t_buf.bitcast(BF16), v_buf.bitcast(BF16)
    cols = pl.ds(0, LANES), pl.ds(LANES, W - LANES)
    fixed = _from(0)

    def read(row, slab, n, sem, halves=(0, 1)):
        return [pltpu.make_async_copy(
            x_hbm.at[pl.ds(row, n), :, cols[h]],
            (x_lo16, x_hi16)[h].at[pl.ds(slab, n)], sem) for h in halves]

    def write(row, n):
        return [pltpu.make_async_copy(
            (o_lo16, o_hi16)[h].at[pl.ds(row, n)],
            o_hbm.at[pl.ds(row, n), :, cols[h]], write_sem) for h in (0, 1)]

    def start(copies, priority=0):
        for c in copies:
            c.start(priority=priority)

    def wait(copies):
        for c in copies:
            c.wait()

    def transform_filter():
        eye = (lax.broadcasted_iota(jnp.int32, (C, C), 0)
               == lax.broadcasted_iota(jnp.int32, (C, C), 1)).astype(BF16)

        def transposed(parts):
            return lax.dot_general(
                eye, jnp.concatenate(parts, axis=0), (((1,), (1,)), ((), ())),
                preferred_element_type=F32)

        def tap(i, kw, rows=slice(None)):
            return x_hi16[X_FILTER + 3 * (2 - i) + kw, rows, :]

        def keep(s, value):
            _store_bf16(v_buf16, fixed, V_FILTER + s, slice(None), value)

        for e in range(2):
            f = [transposed([tap(i, 0, pl.ds(32 * e, 32)), tap(i, 1 + e)])
                 for i in range(3)]
            for j in range(6):
                keep(2 * j + e, functools.reduce(jnp.add, [
                    f[i] * float(G[j, i]) for i in (0, 2, 1) if G[j, i] != 0.0]))
        direct = [tap(i, 0, pl.ds(64, 32)) for i in range(3)]
        pad = [jnp.zeros((32, C), BF16)]
        keep(12, transposed(direct + pad))
        keep(13, transposed(pad + direct))

    def transform_tile(n, i, x_row):
        owner = [None] * LANES
        for g, a, b in _pieces(n):
            for c in range(a - 2, b):
                owner[c % LANES] = (LANES <= c < W, 4 * g + (X_WRAP if c >= W else 0))

        def load(q, key):
            return (x_hi if key[0] else x_lo)[x_row(key[1] + q), _words(i), :]

        d = [_merge(owner, functools.partial(load, q)) for q in range(6)]
        t = _input_transform([_as_bf16(v).astype(F32) for v in d])

        def store(index):
            base = 8 * (n % 3)
            for j in range(6):
                _store_bf16(t_buf16, index, base + j, _chans(i), t[j])
            if i >= 4:
                for q in range(6):
                    rows = _words(2 * (q % 3) + i - 4)
                    t_buf[_slab(index, base + 6 + q // 3, rows)] = d[q]
        return store

    def gather_row(row, i, index, o_row):
        *pieces, (last, begin, stop) = [
            (n, a, b) for n in range(NUM_TILES)
            for g, a, b in _pieces(n) if g == row // 4]
        wrapped, high = [None] * LANES, pieces[-1][0]
        for n, a, b in pieces:
            for c in range(max(a, W), b):
                wrapped[c % LANES] = n
        kept = {}

        def load(n):
            if n not in kept:
                s = 4 * (n % PERIOD_TILES) + row % 4
                kept[n] = v_buf[_slab(index, s, _words(i))]
            return kept[n]

        def roll():
            kept["rolled"] = pltpu.roll(_merge(wrapped, load), 2 * LANES - W, 1)
            o_hi[o_row(row), _words(i), :] = kept.pop(high)[:, :W - LANES]

        def store():
            owner = (["rolled"] * begin + [None] * (stop - begin)
                     + [high] * (LANES - stop))
            o_lo[o_row(row), _words(i), :] = _merge(owner, load)

        def finish():
            o_lo[o_row(row), _words(i), begin:stop] = load(last)[:, begin:stop]
        return roll, store, finish

    def run_block(first, end, rep, read_sems, zeros):
        periods = rep * ((end - first) // PERIOD_TILES)
        ld, st = [_from(z) for z in zeros]
        row_ld, row_st = [_from(periods * (4 * PERIOD_GROUPS) + z) for z in zeros]
        work, val = [], {}
        DOT, STORE, COPY, LOAD = range(4)

        def at(step, kind, *args):
            def register(fn):
                rel = min(step, STEPS * end) - STEPS * first
                key = (rel, kind, 0) if rel >= 0 else (-1, 0, rel)
                work.append((key, len(work), functools.partial(fn, *args)))
            return register

        def fence(step, v, stored):
            v, rows = _as_u32(v[:8]), _words(step % 6)
            if step % 2 == 0:
                t_buf[_slab(st, T_FENCE, rows)] = v
                x_lo[st(X_FENCE_LO), rows, :] = v
            elif not stored:
                v_buf[_slab(st, V_FENCE, rows)] = v
            if (step + 1) % STEPS in TRANSFORM_AT:
                x_hi[st(X_FENCE_HI), rows, :] = v[:, :W - LANES]

        def filter_rows(name, step, slabs):
            for i in range(6):
                @at(step - LEAD_FILTER + i, LOAD, i)
                def _(i):
                    val[name, i] = jnp.concatenate(
                        [v_buf16[_slab(ld, s, _chans(i))] for s in slabs], axis=1)
            return lambda: jnp.concatenate([val[name, i] for i in range(6)], axis=0)

        def product(n, j, step):
            src = 8 * (n % 3) + j
            for q, i in enumerate(reversed(range(6))):
                if n == first and j in PRE_ROLLED:
                    @at(step - LEAD_RAW, LOAD, i)
                    def _(i):
                        val["rolled", n, j, i] = [
                            t_buf16[_slab(ld, T_ROLLED + 2 * j + e, _chans(i))]
                            for e in range(2)]
                else:
                    @at(step - LEAD_ROLL + q, LOAD, i)
                    def _(i):
                        v = t_buf[_slab(ld, src, _words(i))]
                        val["rolled", n, j, i] = [
                            _as_bf16(pltpu.roll(v, 1 + e, 1)) for e in range(2)]
                if n == end - 1 and j in PRE_ROLLED:
                    @at(step + STEPS - LEAD_ROLL + q, LOAD, i)
                    def _(i):
                        v = t_buf[_slab(ld, 8 * (end % 3) + j, _words(i))]
                        val["next", j, i] = [pltpu.roll(v, 1 + e, 1) for e in range(2)]

                    @at(step + STEPS - LEAD_ROLL + q + ROLL_DELAY, STORE, i)
                    def _(i):
                        for e, v in enumerate(val["next", j, i]):
                            t_buf[_slab(st, T_ROLLED + 2 * j + e, _words(i))] = v

            @at(step - LEAD_PLAIN, LOAD)
            def _():
                val["plain", n, j] = t_buf16[_slab(ld, src, pl.ds(0, 64))]

            lhs = filter_rows(
                ("u", n, j), step, [V_FILTER + 2 * j + e for e in range(2)])

            @at(step, DOT)
            def _():
                rhs = []
                for e in range(2):
                    rhs.append(val["plain", n, j][32 * e:32 * e + 32])
                    rhs += [val["rolled", n, j, i][e] for i in range(6)]
                val["m", n, j] = jnp.dot(
                    lhs(), jnp.concatenate(rhs, axis=0), preferred_element_type=F32)

        def direct(n, k, step):
            @at(step - LEAD_RAW, LOAD)
            def _():
                val["raw", n, k] = jnp.concatenate([
                    t_buf16[_slab(ld, 8 * (n % 3) + 6 + q // 3, pl.ds(32 * (q % 3), 32))]
                    for q in range(k, k + 4)], axis=0)

            for e in range(2):
                lhs = filter_rows(("r", n, k + e), step, [V_FILTER + 12 + e])

                @at(step, DOT, e, lhs)
                def _(e, lhs):
                    val["d", n, k + e] = jnp.dot(
                        lhs(), val["raw", n, k], preferred_element_type=F32)

        def output_transform(n, i):
            t0 = STEPS * n
            partial = [O_PARTIAL + 2 * e + i // 3 for e in range(2)]
            rows = pl.ds(16 * (i % 3), 16)

            def result(kind, j):
                return val[kind, n, j][16 * i:16 * i + 16]

            def put(k, y):
                _store_bf16(v_buf16, st, 4 * (n % PERIOD_TILES) + k, _chans(i), y)

            @at(t0 + i, STORE)
            def _():
                m1, m2 = result("m", 1), result("m", 2)
                val["st", n, i] = m1 + m2, m1 - m2
                fence(i, m1, False)

            @at(t0 + 6 + i, STORE)
            def _():
                m3, m4 = result("m", 3), result("m", 4)
                s, t = val["st", n, i]
                u, v = m3 + m4, m3 - m4
                z = s + u
                val["p01", n, i] = z + s, B * (t + v)
                o_lo[st(partial[0]), rows, :] = _as_u32(z + u)
                fence(6 + i, m3, False)
                o_lo[st(partial[1]), rows, :] = _as_u32(A * (t + 4.0 * v))

            @at(t0 + 12 + i, STORE)
            def _():
                p0, p1 = val["p01", n, i]
                put(0, (p0 + result("d", 0)) + result("m", 0))
                y1 = p1 + result("d", 1)
                put(1, y1)
                fence(12 + i, y1, True)

            @at(t0 + 18 + i - LEAD_PARTIAL, LOAD)
            def _():
                val["p23", n, i] = [
                    pltpu.bitcast(o_lo[ld(s), rows, :], F32) for s in partial]

            @at(t0 + 18 + i, STORE)
            def _():
                p2, p3 = val["p23", n, i]
                y2 = p2 + result("d", 2)
                put(2, y2)
                fence(18 + i, y2, True)
                put(3, (p3 + result("d", 3)) + result("m", 5))

        for n in range(first, end):
            t0 = STEPS * n
            product(n, 1, t0)
            product(n, 2, t0)
            product(n, 3, t0 + 6)
            product(n, 4, t0 + 6)
            product(n, 0, t0 + 12)
            direct(n, 0, t0 + 12)
            product(n, 5, t0 + 18)
            direct(n, 2, t0 + 18)
            for i in range(6):
                output_transform(n, i)
            for step, i in zip(TRANSFORM_AT, reversed(range(6))):
                @at(t0 + step, LOAD, n, i)
                def _(n, i):
                    val["t", n, i] = transform_tile(n + 2, i, row_ld)

                @at(t0 + step + TRANSFORM_DELAY, STORE, n, i)
                def _(n, i):
                    val["t", n, i](st)

        for g in range(2, NUM_GROUPS + 2):
            begin = _group_step(g, WRAP_AT)
            if STEPS * first <= begin < STEPS * end:
                length = WRAP_LEN[(g - 1) % PERIOD_GROUPS]
                for k in range(4):
                    for i in range(6):
                        step = begin + ((5 - i) * 4 + k) * length // 24

                        @at(step, LOAD, 4 * g + 2 + k, i)
                        def _(s, i):
                            val["wrap", s, i] = pltpu.roll(
                                x_lo[row_ld(s), _words(i), :], W - LANES, 1)

                        @at(step + ROLL_DELAY, STORE, 4 * g + 2 + k, i)
                        def _(s, i):
                            x_lo[row_st(X_WRAP + s), _words(i), :] = val["wrap", s, i]

        for row in range(H):
            if STEPS * first <= _gather_step(row - row % 2, 0) < STEPS * end:
                for i in range(6):
                    roll, store, _ = gather_row(row, i, ld, row_st)
                    at(_gather_step(row, i), LOAD)(roll)
                    at(_gather_step(row, i) + ROLL_DELAY, LOAD)(store)
            if STEPS * first <= _finish_step(row, 0) < STEPS * end:
                for i in range(6):
                    at(_finish_step(row, i), LOAD)(gather_row(row, i, ld, row_st)[2])

        for q, (n, s, block) in enumerate(READS):
            if first <= n < end:
                @at(STEPS * n + COPY_AT, COPY, q, s, block)
                def _(q, s, block):
                    start(read(s - 2, s, 1, read_sems.at[block]), priority=q % 2)

        for q, (n, _) in enumerate(WRITES):
            if first <= n < end:
                @at(STEPS * n + COPY_AT, COPY, q)
                def _(q):
                    start(write(scalars[periods * WRITES_PER_PERIOD + (2 + q)], 1))

        for _, _, fn in sorted(work, key=lambda item: item[:2]):
            fn()

    def compute(read_sems, first_sems):
        def block_rows(block):
            copies = []
            for half, edges in enumerate(READ_EDGES):
                s, n = edges[block], edges[block + 1] - edges[block]
                copies += read(s - 2, s, n, read_sems.at[block], [half])
            return copies

        def wrap(slabs):
            for s in slabs:
                x_lo[X_WRAP + s] = pltpu.roll(x_lo[s], W - LANES, 1)

        first_rows = (read(H - 2, 0, 2, first_sems.at[0])
                      + read(0, 2, 4, first_sems.at[0]))
        taps = [pltpu.make_async_copy(
            w_hbm, x_hi16.at[pl.ds(X_FILTER, 9)], first_sems.at[1])]
        taps += read(4, 6, 4, first_sems.at[1], [0])
        start(first_rows + taps)
        for block in range(BULK_READS):
            start(block_rows(block))
        scalars[0] = 0
        scalars[1] = 0
        for q, (_, row) in enumerate(WRITES):
            scalars[2 + q] = row
        for s in range(H + 2, X_SLABS):
            x_lo[s] = jnp.zeros(x_lo.shape[1:], U32)
            x_hi[s] = jnp.zeros(x_hi.shape[1:], U32)

        wait(first_rows)
        wrap(range(6))
        for s in range(2):
            x_lo[H + s] = x_lo[s]
            x_hi[H + s] = x_hi[s]
        for n in range(2):
            for i in range(6):
                transform_tile(n, i, fixed)(fixed)
        wait(taps)
        wrap(range(6, 10))
        for j in PRE_ROLLED:
            for e in range(2):
                t_buf[_slab(fixed, T_ROLLED + 2 * j + e, slice(None))] = pltpu.roll(
                    t_buf[_slab(fixed, j, slice(None))], 1 + e, 1)
        transform_filter()

        zeros = scalars[0], scalars[1]
        first = 0
        for block, (tiles, _) in enumerate(BLOCKS[:-1]):
            wait(block_rows(block))
            run_block(first, first + tiles, 0, read_sems, zeros)
            first += tiles
        for row in FIRST_WRITES:
            start(write(row, 1))
        tiles, reps = BLOCKS[-1]

        @pl.loop(0, reps)
        def _(rep):
            for i in range(reps):
                pl.when(rep == i)(lambda: wait(block_rows(len(BLOCKS) - 1 + i)))
            run_block(first, first + tiles, rep, read_sems, zeros)

        start(write(H - 4, 4))

    pl.run_scoped(compute, pltpu.SemaphoreType.DMA((len(ENDS),)),
                  pltpu.SemaphoreType.DMA((2,)))
    wait(write(0, H))


@jax.jit
def pallas_standalone__fft_conv__vision_kernel(x: jax.Array, w: jax.Array):
    assert x.shape == (1, H, W, C) and w.shape == (3, 3, C, C)
    y = pl.pallas_call(
        _kernel,
        in_specs=[pl.BlockSpec(memory_space=pl.ANY)] * 2,
        out_specs=pl.BlockSpec(memory_space=pl.ANY),
        out_shape=jax.ShapeDtypeStruct((H, C, W), BF16),
        scratch_shapes=[
            pltpu.VMEM((2 * X_SLABS + 2, C, LANES), BF16),
            pltpu.VMEM((X_SLABS + 10, C, W - LANES), BF16),
            pltpu.VMEM((H + 4, C, LANES), BF16),
            pltpu.VMEM((H, C, W - LANES), BF16),
            pltpu.VMEM((T_FENCE // 2 + 1, C // 2, 2 * LANES), U32),
            pltpu.VMEM((V_FENCE // 2 + 1, C // 2, 2 * LANES), U32),
            pltpu.SMEM((2 + len(WRITES),), jnp.int32),
            pltpu.SemaphoreType.DMA(()),
        ],
        compiler_params=pltpu.CompilerParams(
            vmem_limit_bytes=64 * 2**20, disable_bounds_checks=True),
    )(x.transpose(0, 1, 3, 2).reshape(H, C, W), w.reshape(9, C, C))
    return y.reshape(1, H, C, W).transpose(0, 1, 3, 2)
```
